```python
import os as _os
_os.environ.setdefault('JAX_PLATFORMS', 'cpu')
import jax
import jax.numpy as jnp

def _softmax(x, axis=-1):
    return jax.nn.softmax(x, axis=axis)

def _gelu(x):
    return jax.nn.gelu(x, approximate=True)

def _silu(x):
    return jax.nn.silu(x)

def _sigmoid(x):
    return jax.nn.sigmoid(x)

def _layernorm(x, axis=-1, eps=1e-05):
    m = jnp.mean(x, axis=axis, keepdims=True)
    v = jnp.var(x, axis=axis, keepdims=True)
    return (x - m) / jnp.sqrt(v + eps)

def _scatter_add(tgt, idx, src, axis=0):
    return tgt.at[idx].add(src)

def _segment_sum(src, seg, n):
    return jax.ops.segment_sum(src, seg, n)

class _Rng:

    def __init__(self, key):
        self._k = key

    def _next(self):
        self._k, sub = jax.random.split(self._k)
        return sub

    def normal(self, shape):
        return jax.random.normal(self._next(), shape, dtype=jnp.bfloat16)

    def randint(self, lo, hi, shape):
        return jax.random.randint(self._next(), shape, lo, hi, dtype=jnp.int32)

    def uniform(self, shape, lo=0.0, hi=1.0):
        return jax.random.uniform(self._next(), shape, jnp.bfloat16, lo, hi)

    def permutation(self, n):
        return jax.random.permutation(self._next(), n)
kernel_name = 'adaLN_cond__ssm_conv_h3__moe_arch_mod__prompt'

def setup_inputs():
    _rng = _Rng(jax.random.key(int.from_bytes(__import__("os").urandom(4), "little")))
    _w = lambda a: (lambda t: t.astype(jnp.bfloat16) if jnp.issubdtype(t.dtype, jnp.floating) else t)(jnp.asarray(a))

    def _A_setup():
        B, S, D = (1, 2048, 640)
        ks = 4
        return {'q': _w((lambda *s: _rng.normal(s) * 0.05)(B, S, D)), 'k': _w((lambda *s: _rng.normal(s) * 0.4)(B, S, D)), 'v': _w((lambda *s: _rng.normal(s) * 0.4)(B, S, D)), 'shift_k': _w((lambda *s: _rng.normal(s) * 0.4)(D, ks) * 0.5), 'ssm_k': _w((lambda *s: _rng.normal(s) * 0.4)(D, S) * (1.0 / S ** 0.5)), 'ssm_D': _w((lambda *s: _rng.normal(s) * 0.4)(D))}
    _A_in = _A_setup()

    def _B_setup():
        B, S, D, F, C = (1, 2048, 640, 1728, 2)
        return {'x': _w((lambda *s: _rng.normal(s) * 0.05)(B, S, D)), 'w_r': _w((lambda *s: _rng.normal(s) * 0.1)(D)), 'w_gate': _w((lambda *s: _rng.normal(s) * 0.1)(D, F)), 'w_up': _w((lambda *s: _rng.normal(s) * 0.1)(D, F)), 'w_down': _w((lambda *s: _rng.normal(s) * 0.1)(F, D))}
    _B_in = _B_setup()
    return {'A_q': _A_in['q'], 'A_k': _A_in['k'], 'A_v': _A_in['v'], 'A_shift_k': _A_in['shift_k'], 'A_ssm_k': _A_in['ssm_k'], 'A_ssm_D': _A_in['ssm_D'], 'B_x': _B_in['x'], 'B_w_r': _B_in['w_r'], 'B_w_gate': _B_in['w_gate'], 'B_w_up': _B_in['w_up'], 'B_w_down': _B_in['w_down'], 'c': _w((lambda *s: _rng.normal(s) * 0.2)(1, 640) * 8.0), 'w_mod': _w((lambda *s: _rng.normal(s) * 0.2)(640, 6 * 640) * 640 ** (-0.5) * 8.0)}

def reference(A_q, A_k, A_v, A_shift_k, A_ssm_k, A_ssm_D, B_x, B_w_r, B_w_gate, B_w_up, B_w_down, c, w_mod):

    def _A_ref(q, k, v, shift_k, ssm_k, ssm_D):
        B, S, D = q.shape
        ks = shift_k.shape[-1]
        k_pad = jnp.pad(k, ((0, 0), (ks - 1, 0), (0, 0)))
        k_shift = jnp.zeros_like(k)
        for t in range(ks):
            k_shift = k_shift + k_pad[:, t:t + S, :] * shift_k[:, ks - 1 - t][None, None, :]
        kv = k_shift * v
        L = 2 * S
        kv_pad = jnp.pad(kv, ((0, 0), (0, S), (0, 0)))
        kf_pad = jnp.pad(ssm_k, ((0, 0), (0, S)))
        kv_f = (lambda x, axes=(-2, -1): jnp.fft.rfft2(x.astype(jnp.float32), axes=axes))(kv_pad[:, None, :, :], axes=(1, 2))
        kf_f = (lambda x, axes=(-2, -1): jnp.fft.rfft2(x.astype(jnp.float32), axes=axes))(kf_pad[:, None, :], axes=(1, 2))
        kf_f = (lambda x, *d: x.transpose(*d))(kf_f, 1, 2, 0)
        y_f = kv_f * kf_f[None, :, :, :]
        y = (lambda x, s, axes=(-2, -1): jnp.fft.irfft2(x, s=s, axes=axes).astype(jnp.bfloat16))(y_f, (1, L), axes=(1, 2))[:, 0, :S, :]
        y = y + kv * ssm_D[None, None, :]
        return q * y

    def _B_ref(x, w_r, w_gate, w_up, w_down):
        B, S, D = x.shape
        C = 2
        r = x @ w_r
        idx = jnp.argsort(-r, axis=-1)[:, :C]
        idx_e = jnp.repeat(idx.reshape(B, C, 1), D, axis=2)
        x_sel = jnp.take_along_axis(x, idx_e, axis=1)
        g = _silu(x_sel @ w_gate)
        u = x_sel @ w_up
        y = g * u @ w_down
        r_sel = _sigmoid(jnp.take_along_axis(r, idx, axis=1))
        y = y * r_sel.reshape(B, C, 1)
        b_off = (jnp.arange(B) * S).reshape(B, 1)
        flat_idx = (idx + b_off).reshape(B * C)
        zero = (x * 0.0).reshape(B * S, D)
        upd = _scatter_add(zero, flat_idx, y.reshape(B * C, D), axis=0)
        return x + upd.reshape(B, S, D)
    x = A_q
    mod = (_silu(c) @ w_mod).reshape(c.shape[0], 6, 1, -1)
    sa, ca, ga, sb, cb, gb = (mod[:, 0].copy(), mod[:, 1].copy(), mod[:, 2].copy(), mod[:, 3].copy(), mod[:, 4].copy(), mod[:, 5].copy())
    h = _layernorm(x, axis=-1) * (1 + ca) + sa
    x = x + ga * _A_ref(h, A_k, A_v, A_shift_k, A_ssm_k, A_ssm_D)
    h = _layernorm(x, axis=-1) * (1 + cb) + sb
    x = x + gb * _B_ref(h, B_w_r, B_w_gate, B_w_up, B_w_down)
    return x
```

```python
import functools

import jax
import jax.numpy as jnp
import numpy as np
import jax.experimental.pallas as pl
import jax.experimental.pallas.tpu as pltpu

S = 2048
D = 640
FF = 1728
NG = D // 128
NB = 4
BLK = S // NB
R = 4
M = BLK // R
MT = M // 8
EPS = 1e-5
NSEM_IN = 3 * NG + 5
f32 = jnp.float32
bf16 = jnp.bfloat16


def _dot(a, b):
    return jnp.dot(a, b, preferred_element_type=f32)


def _dot_nt(a, b):
    return jax.lax.dot_general(a, b, (((1,), (1,)), ((), ())),
                               preferred_element_type=f32)


def _bfly(tr, ti, sign):
    s0r, s0i = tr[0] + tr[2], ti[0] + ti[2]
    d0r, d0i = tr[0] - tr[2], ti[0] - ti[2]
    s1r, s1i = tr[1] + tr[3], ti[1] + ti[3]
    d1r, d1i = tr[1] - tr[3], ti[1] - ti[3]
    pr, pi = d0r - d1i, d0i + d1r
    mr, mi = d0r + d1i, d0i - d1r
    if sign > 0:
        return ([s0r + s1r, pr, s0r - s1r, mr], [s0i + s1i, pi, s0i - s1i, mi])
    return ([s0r + s1r, mr, s0r - s1r, pr], [s0i + s1i, mi, s0i - s1i, pi])


def _kernel(q_hbm, k_hbm, v_hbm, sh_hbm, sk_hbm, dd_hbm, wr_hbm, wg_hbm, wu_hbm,
            wd_hbm, c_hbm, wm_hbm, o_hbm,
            kb, vb, skb, qb, wmb, wgb, wub, wdb, shb, ddb, wrb, cb,
            kf, kvf, skt, xs, ks, ub, yb, h2b, ob, fm, gm, modb,
            st, rb, sem):
    small = [pltpu.make_async_copy(s, t, sem.at[NSEM_IN + i]) for i, (s, t) in
             enumerate([(sh_hbm, shb), (dd_hbm, ddb), (wr_hbm, wrb), (c_hbm, cb)])]

    def conv_copies(g):
        cols = pl.ds(g * 128, 128)
        return [
            pltpu.make_async_copy(k_hbm.at[:, cols], kb.at[g], sem.at[3 * g]),
            pltpu.make_async_copy(v_hbm.at[:, cols], vb.at[g], sem.at[3 * g + 1]),
            pltpu.make_async_copy(sk_hbm.at[cols, :], skb.at[g], sem.at[3 * g + 2]),
        ]

    n0 = 3 * NG
    cp_wm = pltpu.make_async_copy(wm_hbm, wmb, sem.at[n0])
    cp_q = pltpu.make_async_copy(q_hbm, qb, sem.at[n0 + 1])
    cp_wg = pltpu.make_async_copy(wg_hbm, wgb, sem.at[n0 + 2])
    cp_wu = pltpu.make_async_copy(wu_hbm, wub, sem.at[n0 + 3])
    cp_wd = pltpu.make_async_copy(wd_hbm, wdb, sem.at[n0 + 4])

    for cp in conv_copies(0):
        cp.start()
    for cp in small:
        cp.start()
    for g in range(1, NG):
        for cp in conv_copies(g):
            cp.start()
    for cp in (cp_wm, cp_q, cp_wg, cp_wu, cp_wd):
        cp.start()

    mi = jax.lax.broadcasted_iota(jnp.int32, (M, M), 0)
    ni = jax.lax.broadcasted_iota(jnp.int32, (M, M), 1)
    th0 = (((4 * mi + 1) * (4 * ni)) & 2047).astype(f32) * (np.pi / 1024)
    c0, s0 = jnp.cos(th0), jnp.sin(th0)
    th1 = (4 * mi + 1).astype(f32) * (np.pi / 1024)
    c1, s1 = jnp.cos(th1), jnp.sin(th1)
    cq, sq = c0, s0
    for q in range(R):
        if q > 0:
            cq, sq = cq * c1 - sq * s1, cq * s1 + sq * c1
        full = jnp.concatenate(
            [cq.reshape(MT, 1, 8, M), sq.reshape(MT, 1, 8, M)], axis=1).reshape(2 * M, M)
        fm[q] = full.astype(bf16)
        gm[q] = (full.T * (1.0 / BLK)).astype(bf16)

    kf[pl.ds(0, 8), :] = jnp.zeros((8, 128), f32)
    for cp in small:
        cp.wait()

    def conv_group(g):
        for cp in conv_copies(g):
            cp.wait()
        sh = shb[:, pl.ds(g * 128, 128)].astype(f32)
        dvec = ddb[pl.ds(g, 1), :].astype(f32)
        CH = 256
        for c in range(S // CH):
            kf[pl.ds(8 + c * CH, CH), :] = kb[g, pl.ds(c * CH, CH), :].astype(f32)
        for c in range(S // CH):
            acc = kf[pl.ds(8 + c * CH, CH), :] * sh[0:1, :]
            for t in range(1, 4):
                acc = acc + kf[pl.ds(8 + c * CH - t, CH), :] * sh[t:t + 1, :]
            kvf[pl.ds(c * CH, CH), :] = acc * vb[g, pl.ds(c * CH, CH), :].astype(f32)
        for c in range(S // 512):
            skt[pl.ds(c * 512, 512), :] = skb[g, :, pl.ds(c * 512, 512)].T.astype(f32)

        for src, dst in ((skt, ks), (kvf, xs)):
            for a in range(NB):
                tr, ti = [], []
                for q in range(R):
                    w = src[pl.ds(a * BLK + q, M, stride=R), :].astype(bf16)
                    t = _dot(fm[q], w).reshape(MT, 2, 8, 128)
                    tr.append(t[:, 0])
                    ti.append(t[:, 1])
                xr, xi = _bfly(tr, ti, +1)
                for p in range(R):
                    dst[:, (a * R + p) * 2] = xr[p]
                    dst[:, (a * R + p) * 2 + 1] = xi[p]

        def mac(mt, carry):
            zr = [[None] * R for _ in range(NB)]
            zi = [[None] * R for _ in range(NB)]
            for p in range(R):
                xr = [xs[mt, (a * R + p) * 2] for a in range(NB)]
                xi = [xs[mt, (a * R + p) * 2 + 1] for a in range(NB)]
                kr0 = [ks[mt, (a * R + p) * 2] for a in range(NB)]
                ki0 = [ks[mt, (a * R + p) * 2 + 1] for a in range(NB)]
                kr = [kr0[0] + dvec] + [kr0[j] + ki0[j - 1] for j in range(1, NB)]
                ki = [ki0[0]] + [ki0[j] - kr0[j - 1] for j in range(1, NB)]
                for a in range(NB):
                    re = im = None
                    for j in range(a + 1):
                        t_re = kr[j] * xr[a - j] - ki[j] * xi[a - j]
                        t_im = kr[j] * xi[a - j] + ki[j] * xr[a - j]
                        re = t_re if re is None else re + t_re
                        im = t_im if im is None else im + t_im
                    zr[a][p], zi[a][p] = re, im
            for a in range(NB):
                ur, ui = _bfly(zr[a], zi[a], -1)
                for q in range(R):
                    ub[a * R + q, mt] = jnp.concatenate([ur[q], ui[q]], axis=0).astype(bf16)
            return carry

        jax.lax.fori_loop(0, MT, mac, 0)

        for a in range(NB):
            for q in range(R):
                u = ub[a * R + q].reshape(2 * M, 128)
                yb[g, pl.ds(a * BLK + q, M, stride=R), :] = _dot(gm[q], u)

    for g in range(NG):
        conv_group(g)

    cp_wm.wait()
    cvec = cb[...].astype(f32)
    sc = (cvec * jax.nn.sigmoid(cvec)).astype(bf16)
    mod = _dot(jnp.broadcast_to(sc, (16, D)), wmb[...])[0:8]
    mod = mod.astype(bf16).astype(f32)
    sa, ca, ga, sb, cbm, gb = [mod[:, i * D:(i + 1) * D] for i in range(6)]
    modb[0] = ga * (1.0 + ca)
    modb[1] = ga * sa
    modb[2] = 1.0 + cbm
    modb[3] = sb
    modb[4] = gb

    cp_q.wait()
    RC = 16

    def lanes(g):
        return pl.ds(g * 128, 128)

    def xload(rows):
        return [qb[rows, lanes(g)].astype(f32) for g in range(NG)]

    def rowsum(parts):
        s = parts[0]
        for t in parts[1:]:
            s = s + t
        return jnp.broadcast_to(jnp.sum(s, axis=-1, keepdims=True), s.shape)

    def mrow(i, g):
        m = modb[i, :, lanes(g)]
        return jnp.concatenate([m] * (RC // 8), axis=0)

    chunks = [pl.ds(c * RC, RC) for c in range(S // RC)]
    for rows in chunks:
        st[0, rows, :] = rowsum(xload(rows)) * (1.0 / D)
    for rows in chunks:
        m1 = st[0, rows, :]
        d = [x - m1 for x in xload(rows)]
        st[1, rows, :] = jax.lax.rsqrt(rowsum([t * t for t in d]) * (1.0 / D) + EPS)
    for rows in chunks:
        m1, rs1 = st[0, rows, :], st[1, rows, :]
        x1 = []
        for g, x in enumerate(xload(rows)):
            t = x + (((x - m1) * rs1) * mrow(0, g) + mrow(1, g)) * yb[g, rows, :]
            yb[g, rows, :] = t
            x1.append(t)
        st[2, rows, :] = rowsum(x1) * (1.0 / D)
    for rows in chunks:
        m2 = st[2, rows, :]
        d = [yb[g, rows, :] - m2 for g in range(NG)]
        st[3, rows, :] = jax.lax.rsqrt(rowsum([t * t for t in d]) * (1.0 / D) + EPS)
    wr = jnp.concatenate([wrb[pl.ds(g, 1), :] for g in range(NG)], axis=1)
    wr16 = jnp.broadcast_to(wr, (16, D))
    for c, rows in enumerate(chunks):
        m2, rs2 = st[2, rows, :], st[3, rows, :]
        for g in range(NG):
            x1 = yb[g, rows, :]
            h2 = ((x1 - m2) * rs2) * mrow(2, g) + mrow(3, g)
            h2b[rows, lanes(g)] = h2.astype(bf16)
            ob[rows, lanes(g)] = (x1 + mrow(4, g) * h2).astype(bf16)
        if (c + 1) % (128 // RC) == 0:
            blk = c // (128 // RC)
            rr = _dot_nt(wr16, h2b[pl.ds(blk * 128, 128), :])
            rb[pl.ds(blk, 1), :] = rr[0:1]

    r = rb[...].astype(bf16).astype(f32)
    pos = (jax.lax.broadcasted_iota(jnp.int32, (S // 128, 128), 0) * 128
           + jax.lax.broadcasted_iota(jnp.int32, (S // 128, 128), 1))
    bits = pltpu.bitcast(r, jnp.int32)
    key = jnp.where(bits < 0, bits ^ 0x7FFF0000, bits) | (S - 1 - pos)

    def vmax(t):
        return jnp.max(jnp.max(t, axis=0, keepdims=True), axis=1, keepdims=True)

    k1 = vmax(key)
    k2 = vmax(jnp.where(key == k1, jnp.iinfo(jnp.int32).min, key))

    def decode(kk):
        hi = kk & jnp.int32(-65536)
        val = pltpu.bitcast(jnp.broadcast_to(
            jnp.where(hi < 0, hi ^ 0x7FFF0000, hi), (8, 128)), f32)
        idx = (S - 1) - (kk[0, 0] & 0xFFFF)
        return idx, jax.nn.sigmoid(val)[0:1, 0:1]

    i1, r1 = decode(k1)
    i2, r2 = decode(k2)

    OC = 128
    NOC = S // OC

    def out_copy(c):
        rows = pl.ds(c * OC, OC)
        return pltpu.make_async_copy(ob.at[rows], o_hbm.at[rows], sem.at[NSEM_IN + 4 + c])

    c1 = i1 // OC
    c2 = i2 // OC

    g1 = pl.multiple_of((i1 // 16) * 16, 16)
    g2 = pl.multiple_of((i2 // 16) * 16, 16)
    xsel = jnp.concatenate([h2b[pl.ds(g1, 16), :], h2b[pl.ds(g2, 16), :]], axis=0)
    cp_wg.wait()
    gg = _dot_nt(xsel, wgb[...]).astype(bf16).astype(f32)
    gg = (gg * jax.nn.sigmoid(gg)).astype(bf16).astype(f32)
    cp_wu.wait()
    uu = _dot_nt(xsel, wub[...]).astype(bf16).astype(f32)
    act = (gg * uu).astype(bf16)

    for c in range(NOC):
        @pl.when(jnp.logical_and(c1 != c, c2 != c))
        def _():
            out_copy(c).start()

    cp_wd.wait()
    yy = _dot(act, wdb[...]).astype(bf16).astype(f32)
    rid = jax.lax.broadcasted_iota(jnp.int32, (16, D), 0)
    gbv = modb[4][0:1, :]
    for idx, base, rv, part in ((i1, g1, r1, yy[0:16]), (i2, g2, r2, yy[16:32])):
        gate = rv
        upd = jnp.where(rid == idx - base, part * gate * gbv, 0.0)
        ob[pl.ds(base, 16), :] = (ob[pl.ds(base, 16), :].astype(f32) + upd).astype(bf16)

    for c in range(NOC):
        @pl.when(jnp.logical_or(c1 == c, c2 == c))
        def _():
            out_copy(c).start()

    for c in range(NOC):
        out_copy(c).wait()


@jax.jit
def pallas_adaLN_cond__ssm_conv_h3__moe_arch_mod__prompt_kernel(
    A_q: jax.Array,
    A_k: jax.Array,
    A_v: jax.Array,
    A_shift_k: jax.Array,
    A_ssm_k: jax.Array,
    A_ssm_D: jax.Array,
    B_x: jax.Array,
    B_w_r: jax.Array,
    B_w_gate: jax.Array,
    B_w_up: jax.Array,
    B_w_down: jax.Array,
    c: jax.Array,
    w_mod: jax.Array,
):
    del B_x
    hbm = pl.BlockSpec(memory_space=pltpu.HBM)
    scratch = [
        pltpu.VMEM((NG, S, 128), bf16),
        pltpu.VMEM((NG, S, 128), bf16),
        pltpu.VMEM((NG, 128, S), bf16),
        pltpu.VMEM((S, D), bf16),
        pltpu.VMEM((D, 6 * D), bf16),
        pltpu.VMEM((FF, D), bf16),
        pltpu.VMEM((FF, D), bf16),
        pltpu.VMEM((FF, D), bf16),
        pltpu.VMEM((4, D), bf16),
        pltpu.VMEM((NG, 128), bf16),
        pltpu.VMEM((NG, 128), bf16),
        pltpu.VMEM((1, D), bf16),
        pltpu.VMEM((S + 8, 128), f32),
        pltpu.VMEM((S, 128), f32),
        pltpu.VMEM((S, 128), f32),
        pltpu.VMEM((MT, 2 * NB * R, 8, 128), f32),
        pltpu.VMEM((MT, 2 * NB * R, 8, 128), f32),
        pltpu.VMEM((NB * R, MT, 16, 128), bf16),
        pltpu.VMEM((NG, S, 128), f32),
        pltpu.VMEM((S, D), bf16),
        pltpu.VMEM((S, D), bf16),
        pltpu.VMEM((R, 2 * M, M), bf16),
        pltpu.VMEM((R, M, 2 * M), bf16),
        pltpu.VMEM((5, 8, D), f32),
        pltpu.VMEM((4, S, 128), f32),
        pltpu.VMEM((S // 128, 128), f32),
        pltpu.SemaphoreType.DMA((NSEM_IN + 4 + S // 128,)),
    ]
    out = pl.pallas_call(
        _kernel,
        out_shape=jax.ShapeDtypeStruct((S, D), bf16),
        in_specs=[hbm] * 12,
        out_specs=hbm,
        scratch_shapes=scratch,
        compiler_params=pltpu.CompilerParams(vmem_limit_bytes=100 * 1024 * 1024),
    )(
        A_q.reshape(S, D), A_k.reshape(S, D), A_v.reshape(S, D),
        A_shift_k.T, A_ssm_k, A_ssm_D.reshape(NG, 128), B_w_r.reshape(NG, 128),
        B_w_gate.T, B_w_up.T, B_w_down, c, w_mod,
    )
    return out.reshape(1, S, D)
```

```python
import jax
import jax.numpy as jnp
import numpy as np
import jax.experimental.pallas as pl
import jax.experimental.pallas.tpu as pltpu

S = 2048
D = 640
FF = 1728
NG = D // 128
NB = 4
BLK = S // NB
R = 4
M = BLK // R
MT = M // 8
EPS = 1e-5
NPOS = 8
RC = 512
OC = 256
NOC = S // OC
WD1 = 1408
SEM_BIG = 3 * NG
SEM_SMALL = SEM_BIG + 6
SEM_OUT = SEM_SMALL + 4
NSEM = SEM_OUT + NOC
FLIP = 0x7FFFFFFF - (S - 1)
f32 = jnp.float32
bf16 = jnp.bfloat16
i32 = jnp.int32


def _dot(a, b):
    return jnp.dot(a, b, preferred_element_type=f32)


def _dot_nt(a, b):
    return jax.lax.dot_general(a, b, (((1,), (1,)), ((), ())),
                               preferred_element_type=f32)


def _rbf(x):
    return x.astype(bf16).astype(f32)


def _bfly(tr, ti, sign):
    s0r, s0i = tr[0] + tr[2], ti[0] + ti[2]
    d0r, d0i = tr[0] - tr[2], ti[0] - ti[2]
    s1r, s1i = tr[1] + tr[3], ti[1] + ti[3]
    d1r, d1i = tr[1] - tr[3], ti[1] - ti[3]
    pr, pi = d0r - d1i, d0i + d1r
    mr, mi = d0r + d1i, d0i - d1r
    if sign > 0:
        return ([s0r + s1r, pr, s0r - s1r, mr], [s0i + s1i, pi, s0i - s1i, mi])
    return ([s0r + s1r, mr, s0r - s1r, pr], [s0i + s1i, mi, s0i - s1i, pi])


def _kernel(q_hbm, k_hbm, v_hbm, sh_hbm, sk_hbm, dd_hbm, wr_hbm, wg_hbm, wu_hbm,
            wd_hbm, c_hbm, wm_hbm, o_hbm,
            kb, vb, skb, qb, wmb, wgb, wub, wdb, shb, ddb, wrb, cb,
            kf, kvf, skt, xs, ks, ub, yb, h2b, ob, fm, gm, modb, st, rb, sem):
    small = [pltpu.make_async_copy(s, t, sem.at[SEM_SMALL + i]) for i, (s, t) in
             enumerate([(sh_hbm, shb), (dd_hbm, ddb), (wr_hbm, wrb), (c_hbm, cb)])]

    def lanes(g):
        return pl.ds(g * 128, 128)

    def conv_copies(g):
        return [
            pltpu.make_async_copy(k_hbm.at[:, lanes(g)], kb.at[g], sem.at[3 * g]),
            pltpu.make_async_copy(v_hbm.at[:, lanes(g)], vb.at[g], sem.at[3 * g + 1]),
            pltpu.make_async_copy(sk_hbm.at[lanes(g), :], skb.at[g], sem.at[3 * g + 2]),
        ]

    cp_q = pltpu.make_async_copy(q_hbm, qb, sem.at[SEM_BIG])
    cp_wm = pltpu.make_async_copy(wm_hbm, wmb, sem.at[SEM_BIG + 1])
    cp_wg = pltpu.make_async_copy(wg_hbm, wgb, sem.at[SEM_BIG + 2])
    cp_wu = pltpu.make_async_copy(wu_hbm, wub, sem.at[SEM_BIG + 3])
    wd1, wd2 = pl.ds(0, WD1), pl.ds(WD1, FF - WD1)
    cp_wd1 = pltpu.make_async_copy(wd_hbm.at[wd1], wdb.at[wd1], sem.at[SEM_BIG + 4])
    cp_wd2 = pltpu.make_async_copy(wd_hbm.at[wd2], wdb.at[wd2], sem.at[SEM_BIG + 5])

    for cp in small:
        cp.start()
    for g in range(NG):
        for cp in conv_copies(g):
            cp.start()
    for cp in (cp_q, cp_wm, cp_wg, cp_wu, cp_wd1, cp_wd2):
        cp.start()

    mi = jax.lax.broadcasted_iota(i32, (M, M), 0)
    ni = jax.lax.broadcasted_iota(i32, (M, M), 1)
    th0 = (((4 * mi + 1) * (4 * ni)) & 2047).astype(f32) * (np.pi / 1024)
    c0, s0 = jnp.cos(th0), jnp.sin(th0)
    th1 = (4 * mi + 1).astype(f32) * (np.pi / 1024)
    c1, s1 = jnp.cos(th1), jnp.sin(th1)
    cq, sq = c0, s0
    for q in range(R):
        if q > 0:
            cq, sq = cq * c1 - sq * s1, cq * s1 + sq * c1
        full = jnp.concatenate(
            [cq.reshape(MT, 1, 8, M), sq.reshape(MT, 1, 8, M)], axis=1).reshape(2 * M, M)
        fm[q] = full.astype(bf16)
        gm[q] = (full.T * (1.0 / BLK)).astype(bf16)

    kf[pl.ds(0, 8), :] = jnp.zeros((8, 128), f32)
    for cp in small:
        cp.wait()

    def wait_group(g):
        for cp in conv_copies(g):
            cp.wait()

    def stage_a(g, a):
        sh = shb[:, lanes(g)].astype(f32)
        rows = pl.ds(a * BLK, BLK)
        kf[pl.ds(8 + a * BLK, BLK), :] = kb[g, rows, :].astype(f32)
        acc = kf[pl.ds(8 + a * BLK, BLK), :] * sh[0:1, :]
        for t in range(1, 4):
            acc = acc + kf[pl.ds(8 + a * BLK - t, BLK), :] * sh[t:t + 1, :]
        kvf[rows, :] = acc * vb[g, rows, :].astype(f32)
        skt[rows, :] = skb[g, :, rows].T.astype(f32)

    def stage_b(g, u):
        src, dst = (skt, ks) if u < NB else (kvf, xs)
        a = u % NB
        tr, ti = [], []
        for q in range(R):
            w = src[pl.ds(a * BLK + q, M, stride=R), :].astype(bf16)
            t = _dot(fm[q], w).reshape(MT, 2, 8, 128)
            tr.append(t[:, 0])
            ti.append(t[:, 1])
        xr, xi = _bfly(tr, ti, +1)
        for p in range(R):
            dst[g % 2, (a * R + p) * 2] = xr[p]
            dst[g % 2, (a * R + p) * 2 + 1] = xi[p]

    def stage_c(g, j0):
        mt = pl.ds(j0 * NPOS, NPOS)
        dvec = ddb[pl.ds(g, 1), :].astype(f32)
        b = g % 2
        zr = [[None] * R for _ in range(NB)]
        zi = [[None] * R for _ in range(NB)]
        for p in range(R):
            xr = [xs[b, (a * R + p) * 2, mt] for a in range(NB)]
            xi = [xs[b, (a * R + p) * 2 + 1, mt] for a in range(NB)]
            kr0 = [ks[b, (a * R + p) * 2, mt] for a in range(NB)]
            ki0 = [ks[b, (a * R + p) * 2 + 1, mt] for a in range(NB)]
            kr = [kr0[0] + dvec] + [kr0[j] + ki0[j - 1] for j in range(1, NB)]
            ki = [ki0[0]] + [ki0[j] - kr0[j - 1] for j in range(1, NB)]
            for a in range(NB):
                re = im = None
                for j in range(a + 1):
                    t_re = kr[j] * xr[a - j] - ki[j] * xi[a - j]
                    t_im = kr[j] * xi[a - j] + ki[j] * xr[a - j]
                    re = t_re if re is None else re + t_re
                    im = t_im if im is None else im + t_im
                zr[a][p], zi[a][p] = re, im
        for a in range(NB):
            ur, ui = _bfly(zr[a], zi[a], -1)
            for q in range(R):
                u = jnp.concatenate([ur[q], ui[q]], axis=1).reshape(16 * NPOS, 128)
                ub[a * R + q, pl.ds(j0 * 16 * NPOS, 16 * NPOS), :] = u.astype(bf16)

    def stage_d(g, a):
        for q in range(R):
            yb[g, pl.ds(a * BLK + q, M, stride=R), :] = _dot(gm[q], ub[a * R + q])

    NT = RC // 8
    sel = (jax.lax.broadcasted_iota(i32, (1, 16, 8, 128), 3) // 8
           == jax.lax.broadcasted_iota(i32, (1, 16, 8, 128), 1))

    def t3(x):
        return x.reshape(NT, 8, 128)

    def xload(rows):
        return [t3(qb[rows, lanes(g)].astype(f32)) for g in range(NG)]

    def rowsum(parts):
        s = parts[0]
        for t in parts[1:]:
            s = s + t
        return jnp.broadcast_to(jnp.sum(s, axis=-1, keepdims=True), s.shape)

    def stats(parts, rows, im, iv):
        s1 = rowsum(parts)
        s2 = rowsum([t * t for t in parts])
        m = s1 * (1.0 / D)
        st[im, rows, :] = m.reshape(RC, 128)
        v = (s2 - m * s1).reshape(RC // 128, 16, 8, 128)
        dense = jnp.sum(jnp.where(sel, v, 0.0), axis=1, keepdims=True)
        rs = jax.lax.rsqrt(jnp.maximum(dense * (1.0 / D), 0.0) + EPS)
        rs = jnp.max(jnp.where(sel, rs, 0.0), axis=-1, keepdims=True)
        st[iv, rows, :] = jnp.broadcast_to(rs, v.shape).reshape(RC, 128)

    chunks = [pl.ds(c * RC, RC) for c in range(S // RC)]

    wait_group(0)
    for a in range(NB):
        stage_a(0, a)
    for g in range(NG + 1):
        for u in range(2 * NB):
            if g < NG:
                stage_b(g, u)
            if g > 0 and (2 * u) % NPOS == 0:
                stage_c(g - 1, 2 * u // NPOS)
        if g + 1 < NG:
            wait_group(g + 1)
        if g == NG:
            cp_q.wait()
        for a in range(NB):
            if g > 0:
                stage_d(g - 1, a)
            if g + 1 < NG:
                stage_a(g + 1, a)
        if g == NG:
            for rows in chunks:
                stats(xload(rows), rows, 0, 1)

    cp_wm.wait()
    cvec = cb[...].astype(f32)
    sc = (cvec * jax.nn.sigmoid(cvec)).astype(bf16)
    mod = _rbf(_dot(jnp.broadcast_to(sc, (16, D)), wmb[...])[0:8])
    sa, ca, ga, sb, cbm, gb = [mod[:, i * D:(i + 1) * D] for i in range(6)]
    modb[0] = ga * (1.0 + ca)
    modb[1] = ga * sa
    modb[2] = 1.0 + cbm
    modb[3] = sb
    modb[4] = gb

    def mrow(i, g):
        return modb[i, :, lanes(g)]

    for rows in chunks:
        m1, rs1 = t3(st[0, rows, :]), t3(st[1, rows, :])
        x1 = []
        for g, x in enumerate(xload(rows)):
            t = x + (((x - m1) * rs1) * mrow(0, g) + mrow(1, g)) * t3(yb[g, rows, :])
            yb[g, rows, :] = t.reshape(RC, 128)
            x1.append(t)
        stats(x1, rows, 2, 3)
    for c, rows in enumerate(chunks):
        m2, rs2 = t3(st[2, rows, :]), t3(st[3, rows, :])
        rr = None
        for g in range(NG):
            x1 = t3(yb[g, rows, :])
            h2 = ((x1 - m2) * rs2) * mrow(2, g) + mrow(3, g)
            h2b[g, rows, :] = h2.reshape(RC, 128).astype(bf16)
            ob[rows, lanes(g)] = (x1 + mrow(4, g) * h2).reshape(RC, 128).astype(bf16)
            t = _dot_nt(jnp.broadcast_to(wrb[pl.ds(g, 1), :], (16, 128)), h2b[g, rows, :])
            rr = t if rr is None else rr + t
        rb[pl.ds(c, 1), :] = rr[0:1]

    r = rb[...]
    pos = (jax.lax.broadcasted_iota(i32, r.shape, 0) * RC
           + jax.lax.broadcasted_iota(i32, r.shape, 1))
    bits = jax.lax.bitcast_convert_type(r, i32) & jnp.int32(-S)
    key = jnp.where(bits < 0, bits ^ FLIP, bits) | (S - 1 - pos)

    def vmax(t):
        return jnp.max(jnp.max(t, axis=0, keepdims=True), axis=1, keepdims=True)

    k1 = vmax(key)
    k2 = vmax(jnp.where(key == k1, jnp.iinfo(i32).min, key))

    def decode(kk):
        hi = jnp.broadcast_to(kk & jnp.int32(-S), (8, 128))
        val = jax.lax.bitcast_convert_type(jnp.where(hi < 0, hi ^ FLIP, hi), f32)
        idx = (S - 1) - (kk[0, 0] & (S - 1))
        return jnp.clip(idx, 0, S - 1), jax.nn.sigmoid(val)[0:1, 0:1]

    i1, gate1 = decode(k1)
    i2, gate2 = decode(k2)
    c1 = i1 // OC
    c2 = i2 // OC

    def out_copy(c):
        rows = pl.ds(c * OC, OC)
        return pltpu.make_async_copy(ob.at[rows], o_hbm.at[rows], sem.at[SEM_OUT + c])

    cp_wd1.wait()
    for c in range(NOC):
        @pl.when(jnp.logical_and(c1 != c, c2 != c))
        def _():
            out_copy(c).start()

    g1 = pl.multiple_of((i1 // 16) * 16, 16)
    g2 = pl.multiple_of((i2 // 16) * 16, 16)
    xsel = jnp.concatenate(
        [jnp.concatenate([h2b[g, pl.ds(r0, 16), :] for g in range(NG)], axis=1)
         for r0 in (g1, g2)], axis=0)
    cp_wg.wait()
    gg = _dot_nt(xsel, wgb[...])
    gg = gg * jax.nn.sigmoid(gg)
    cp_wu.wait()
    act = (gg * _dot_nt(xsel, wub[...])).astype(bf16)

    cp_wd2.wait()
    yy = _dot(act, wdb[...])
    rid = jax.lax.broadcasted_iota(i32, (16, D), 0)
    gbv = modb[4][0:1, :]
    for idx, base, gate, part in ((i1, g1, gate1, yy[0:16]), (i2, g2, gate2, yy[16:32])):
        upd = jnp.where(rid == idx - base, part * gate * gbv, 0.0)
        ob[pl.ds(base, 16), :] = (ob[pl.ds(base, 16), :].astype(f32) + upd).astype(bf16)

    for c in range(NOC):
        @pl.when(jnp.logical_or(c1 == c, c2 == c))
        def _():
            out_copy(c).start()

    for c in range(NOC):
        out_copy(c).wait()


@jax.jit
def pallas_adaLN_cond__ssm_conv_h3__moe_arch_mod__prompt_kernel(
    A_q: jax.Array,
    A_k: jax.Array,
    A_v: jax.Array,
    A_shift_k: jax.Array,
    A_ssm_k: jax.Array,
    A_ssm_D: jax.Array,
    B_x: jax.Array,
    B_w_r: jax.Array,
    B_w_gate: jax.Array,
    B_w_up: jax.Array,
    B_w_down: jax.Array,
    c: jax.Array,
    w_mod: jax.Array,
):
    del B_x
    hbm = pl.BlockSpec(memory_space=pltpu.HBM)
    scratch = [
        pltpu.VMEM((NG, S, 128), bf16),
        pltpu.VMEM((NG, S, 128), bf16),
        pltpu.VMEM((NG, 128, S), bf16),
        pltpu.VMEM((S, D), bf16),
        pltpu.VMEM((D, 6 * D), bf16),
        pltpu.VMEM((FF, D), bf16),
        pltpu.VMEM((FF, D), bf16),
        pltpu.VMEM((FF, D), bf16),
        pltpu.VMEM((4, D), bf16),
        pltpu.VMEM((NG, 128), bf16),
        pltpu.VMEM((NG, 128), bf16),
        pltpu.VMEM((1, D), bf16),
        pltpu.VMEM((S + 8, 128), f32),
        pltpu.VMEM((S, 128), f32),
        pltpu.VMEM((S, 128), f32),
        pltpu.VMEM((2, 2 * NB * R, MT, 8, 128), f32),
        pltpu.VMEM((2, 2 * NB * R, MT, 8, 128), f32),
        pltpu.VMEM((NB * R, 2 * M, 128), bf16),
        pltpu.VMEM((NG, S, 128), f32),
        pltpu.VMEM((NG, S, 128), bf16),
        pltpu.VMEM((S, D), bf16),
        pltpu.VMEM((R, 2 * M, M), bf16),
        pltpu.VMEM((R, M, 2 * M), bf16),
        pltpu.VMEM((5, 8, D), f32),
        pltpu.VMEM((4, S, 128), f32),
        pltpu.VMEM((S // RC, RC), f32),
        pltpu.SemaphoreType.DMA((NSEM,)),
    ]
    out = pl.pallas_call(
        _kernel,
        out_shape=jax.ShapeDtypeStruct((S, D), bf16),
        in_specs=[hbm] * 12,
        out_specs=hbm,
        scratch_shapes=scratch,
        compiler_params=pltpu.CompilerParams(vmem_limit_bytes=100 * 1024 * 1024),
    )(
        A_q.reshape(S, D), A_k.reshape(S, D), A_v.reshape(S, D),
        A_shift_k.T, A_ssm_k, A_ssm_D.reshape(NG, 128), B_w_r.reshape(NG, 128),
        B_w_gate.T, B_w_up.T, B_w_down, c, w_mod,
    )
    return out.reshape(1, S, D)
```

```python
import jax
import jax.numpy as jnp
import numpy as np
import jax.experimental.pallas as pl
import jax.experimental.pallas.tpu as pltpu

S = 2048
D = 640
FF = 1728
NG = D // 128
NB = 4
BLK = S // NB
R = 4
M = BLK // R
MT = M // 8
EPS = 1e-5
NPOS = MT // 2
RC = 512
QG = NG + 1 - S // RC
NOC = 8
OR = RC // NOC
WD1 = 1472
SEM_BIG = NG + 2 * NB
SEM_SMALL = SEM_BIG + 6
SEM_OUT = SEM_SMALL + 4
NSEM = SEM_OUT + NOC
FLIP = 0x7FFFFFFF - (S - 1)
f32 = jnp.float32
bf16 = jnp.bfloat16
i32 = jnp.int32


def _dot(a, b):
    return jnp.dot(a, b, preferred_element_type=f32)


def _dot_nt(a, b):
    return jax.lax.dot_general(a, b, (((1,), (1,)), ((), ())),
                               preferred_element_type=f32)


def _rbf(x):
    return x.astype(bf16).astype(f32)


def _bfly(tr, ti, sign):
    s0r, s0i = tr[0] + tr[2], ti[0] + ti[2]
    d0r, d0i = tr[0] - tr[2], ti[0] - ti[2]
    s1r, s1i = tr[1] + tr[3], ti[1] + ti[3]
    d1r, d1i = tr[1] - tr[3], ti[1] - ti[3]
    pr, pi = d0r - d1i, d0i + d1r
    mr, mi = d0r + d1i, d0i - d1r
    if sign > 0:
        return ([s0r + s1r, pr, s0r - s1r, mr], [s0i + s1i, pi, s0i - s1i, mi])
    return ([s0r + s1r, mr, s0r - s1r, pr], [s0i + s1i, mi, s0i - s1i, pi])


def _kernel(q_hbm, k_hbm, v_hbm, sh_hbm, sk_hbm, dd_hbm, wr_hbm, wg_hbm, wu_hbm,
            wd_hbm, c_hbm, wm_hbm, o_hbm,
            kb, vb, skb, qb, wmb, wgb, wub, wdb, shb, ddb, wrb, cb,
            kf, kvf, skt, xs, ks, ub, yb, h2b, ob, fm, gm, modb, st, rb, sem):
    small = [pltpu.make_async_copy(s, t, sem.at[SEM_SMALL + i]) for i, (s, t) in
             enumerate([(sh_hbm, shb), (dd_hbm, ddb), (wr_hbm, wrb), (c_hbm, cb)])]

    def lanes(g):
        return pl.ds(g * 128, 128)

    def blk_rows(a):
        return pl.ds(a * BLK, BLK)

    def sk_copy(g):
        return pltpu.make_async_copy(sk_hbm.at[lanes(g), :], skb.at[g], sem.at[g])

    def kv_copies(a):
        return [
            pltpu.make_async_copy(k_hbm.at[blk_rows(a)], kb.at[blk_rows(a)], sem.at[NG + 2 * a]),
            pltpu.make_async_copy(v_hbm.at[blk_rows(a)], vb.at[blk_rows(a)], sem.at[NG + 2 * a + 1]),
        ]

    cp_q = pltpu.make_async_copy(q_hbm, qb, sem.at[SEM_BIG])
    cp_wm = pltpu.make_async_copy(wm_hbm, wmb, sem.at[SEM_BIG + 1])
    cp_wg = pltpu.make_async_copy(wg_hbm, wgb, sem.at[SEM_BIG + 2])
    cp_wu = pltpu.make_async_copy(wu_hbm, wub, sem.at[SEM_BIG + 3])
    wd1, wd2 = pl.ds(0, WD1), pl.ds(WD1, FF - WD1)
    cp_wd1 = pltpu.make_async_copy(wd_hbm.at[wd1], wdb.at[wd1], sem.at[SEM_BIG + 4])
    cp_wd2 = pltpu.make_async_copy(wd_hbm.at[wd2], wdb.at[wd2], sem.at[SEM_BIG + 5])

    sk_copy(0).start()
    for cp in small:
        cp.start()
    for g in range(1, NG):
        sk_copy(g).start()
    for a in range(NB):
        for cp in kv_copies(a):
            cp.start()
    for cp in (cp_q, cp_wm, cp_wg, cp_wu, cp_wd1, cp_wd2):
        cp.start()

    mi = jax.lax.broadcasted_iota(i32, (M, M), 0)
    ni = jax.lax.broadcasted_iota(i32, (M, M), 1)
    th0 = (((4 * mi + 1) * (4 * ni)) & 2047).astype(f32) * (np.pi / 1024)
    c0, s0 = jnp.cos(th0), jnp.sin(th0)
    th1 = (4 * mi + 1).astype(f32) * (np.pi / 1024)
    c1, s1 = jnp.cos(th1), jnp.sin(th1)
    cq, sq = c0, s0
    for q in range(R):
        if q > 0:
            cq, sq = cq * c1 - sq * s1, cq * s1 + sq * c1
        full = jnp.concatenate(
            [cq.reshape(MT, 1, 8, M), sq.reshape(MT, 1, 8, M)], axis=1).reshape(2 * M, M)
        fm[q] = full.astype(bf16)
        gm[q] = (full.T * (1.0 / BLK)).astype(bf16)

    def prep_k(g):
        for a in range(NB):
            skt[g % 2, blk_rows(a), :] = skb[g, :, blk_rows(a)].T.astype(f32)

    def prep_x(g, a):
        b = g % 2
        sh = shb[:, lanes(g)].astype(f32)
        if a == 0:
            kf[b, pl.ds(0, 16), :] = jnp.zeros((16, 128), f32)
            kf[b, pl.ds(16, BLK), :] = kb[blk_rows(0), lanes(g)].astype(f32)
        else:
            kf[b] = kb[pl.ds(a * BLK - 16, BLK + 16), lanes(g)].astype(f32)
        acc = kf[b, pl.ds(16, BLK), :] * sh[0:1, :]
        for t in range(1, 4):
            acc = acc + kf[b, pl.ds(16 - t, BLK), :] * sh[t:t + 1, :]
        kvf[b] = acc * vb[blk_rows(a), lanes(g)].astype(f32)

    def fwd(src, row0, dst, g, a):
        tr, ti = [], []
        for q in range(R):
            w = src[g % 2, pl.ds(row0 + q, M, stride=R), :].astype(bf16)
            t = _dot(fm[q], w).reshape(MT, 2, 8, 128)
            tr.append(t[:, 0])
            ti.append(t[:, 1])
        xr, xi = _bfly(tr, ti, +1)
        for p in range(R):
            dst[g, (a * R + p) * 2] = xr[p]
            dst[g, (a * R + p) * 2 + 1] = xi[p]

    def stage_c(g, j0):
        mt = pl.ds(j0 * NPOS, NPOS)
        dvec = ddb[pl.ds(g, 1), :].astype(f32)
        zr = [[None] * R for _ in range(NB)]
        zi = [[None] * R for _ in range(NB)]
        for p in range(R):
            xr = [xs[g, (a * R + p) * 2, mt] for a in range(NB)]
            xi = [xs[g, (a * R + p) * 2 + 1, mt] for a in range(NB)]
            kr0 = [ks[g, (a * R + p) * 2, mt] for a in range(NB)]
            ki0 = [ks[g, (a * R + p) * 2 + 1, mt] for a in range(NB)]
            kr = [kr0[0] + dvec] + [kr0[j] + ki0[j - 1] for j in range(1, NB)]
            ki = [ki0[0]] + [ki0[j] - kr0[j - 1] for j in range(1, NB)]
            for a in range(NB):
                re = im = None
                for j in range(a + 1):
                    t_re = kr[j] * xr[a - j] - ki[j] * xi[a - j]
                    t_im = kr[j] * xi[a - j] + ki[j] * xr[a - j]
                    re = t_re if re is None else re + t_re
                    im = t_im if im is None else im + t_im
                zr[a][p], zi[a][p] = re, im
        for a in range(NB):
            ur, ui = _bfly(zr[a], zi[a], -1)
            for q in range(R):
                u = jnp.concatenate([ur[q], ui[q]], axis=1).reshape(16 * NPOS, 128)
                ub[g % 2, a * R + q, pl.ds(j0 * 16 * NPOS, 16 * NPOS), :] = u.astype(bf16)

    def stage_d(g, a):
        for q in range(R):
            yb[g, pl.ds(a * BLK + q, M, stride=R), :] = _dot(gm[q], ub[g % 2, a * R + q])

    NT = RC // 8
    sel = (jax.lax.broadcasted_iota(i32, (1, 16, 8, 128), 3) // 8
           == jax.lax.broadcasted_iota(i32, (1, 16, 8, 128), 1))

    def t3(x):
        return x.reshape(NT, 8, 128)

    def xload(rows):
        return [t3(qb[rows, lanes(g)].astype(f32)) for g in range(NG)]

    def rowsum(parts):
        s = parts[0]
        for t in parts[1:]:
            s = s + t
        return jnp.broadcast_to(jnp.sum(s, axis=-1, keepdims=True), s.shape)

    def stats(parts, rows, im, iv):
        s1 = rowsum(parts)
        s2 = rowsum([t * t for t in parts])
        m = s1 * (1.0 / D)
        st[im, rows, :] = m.reshape(RC, 128)
        v = (s2 - m * s1).reshape(RC // 128, 16, 8, 128)
        dense = jnp.sum(jnp.where(sel, v, 0.0), axis=1, keepdims=True)
        rs = jax.lax.rsqrt(jnp.maximum(dense * (1.0 / D), 0.0) + EPS)
        rs = jnp.max(jnp.where(sel, rs, 0.0), axis=-1, keepdims=True)
        st[iv, rows, :] = jnp.broadcast_to(rs, v.shape).reshape(RC, 128)

    chunks = [pl.ds(c * RC, RC) for c in range(S // RC)]

    for g in range(NG + 1):
        if g < NG:
            sk_copy(g).wait()
        if g > 0:
            for a in range(NB):
                fwd(skt, a * BLK, ks, g - 1, a)
        if g < NG:
            prep_k(g)
    for cp in small:
        cp.wait()
    for a in range(NB):
        for cp in kv_copies(a):
            cp.wait()
        for g in range(NG):
            prep_x(g, a)
            fwd(kvf, 0, xs, g, a)
    for g in range(NG + 1):
        if g == QG:
            cp_q.wait()
        for a in range(NB):
            if g > 0:
                stage_d(g - 1, a)
            if g < NG and a % 2 == 0:
                stage_c(g, a // 2)
        if g >= QG:
            stats(xload(chunks[g - QG]), chunks[g - QG], 0, 1)

    cp_wm.wait()
    cvec = cb[...].astype(f32)
    sc = (cvec * jax.nn.sigmoid(cvec)).astype(bf16)
    mod = _rbf(_dot(jnp.broadcast_to(sc, (16, D)), wmb[...])[0:8])
    sa, ca, ga, sb, cbm, gb = [mod[:, i * D:(i + 1) * D] for i in range(6)]
    modb[0] = ga * (1.0 + ca)
    modb[1] = ga * sa
    modb[2] = 1.0 + cbm
    modb[3] = sb
    modb[4] = gb

    def mrow(i, g):
        return modb[i, :, lanes(g)]

    for rows in chunks:
        m1, rs1 = t3(st[0, rows, :]), t3(st[1, rows, :])
        x1 = []
        for g, x in enumerate(xload(rows)):
            t = x + (((x - m1) * rs1) * mrow(0, g) + mrow(1, g)) * t3(yb[g, rows, :])
            yb[g, rows, :] = t.reshape(RC, 128)
            x1.append(t)
        stats(x1, rows, 2, 3)
    for c, rows in enumerate(chunks):
        m2, rs2 = t3(st[2, rows, :]), t3(st[3, rows, :])
        rr = None
        for g in range(NG):
            x1 = t3(yb[g, rows, :])
            h2 = ((x1 - m2) * rs2) * mrow(2, g) + mrow(3, g)
            h2b[g, rows, :] = h2.reshape(RC, 128).astype(bf16)
            ob[c, :, :, lanes(g)] = (x1 + mrow(4, g) * h2).reshape(NOC, OR, 128).astype(bf16)
            t = _dot_nt(jnp.broadcast_to(wrb[pl.ds(g, 1), :], (16, 128)), h2b[g, rows, :])
            rr = t if rr is None else rr + t
        rb[pl.ds(c, 1), :] = rr[0:1]

    r = _rbf(rb[...])
    pos = (jax.lax.broadcasted_iota(i32, r.shape, 0) * RC
           + jax.lax.broadcasted_iota(i32, r.shape, 1))
    bits = jax.lax.bitcast_convert_type(r, i32) & jnp.int32(-S)
    key = jnp.where(bits < 0, bits ^ FLIP, bits) | (S - 1 - pos)

    def vmax(t):
        return jnp.max(jnp.max(t, axis=0, keepdims=True), axis=1, keepdims=True)

    k1 = vmax(key)
    k2 = vmax(jnp.where(key == k1, jnp.iinfo(i32).min, key))

    def decode(kk):
        hi = jnp.broadcast_to(kk & jnp.int32(-S), (8, 128))
        val = jax.lax.bitcast_convert_type(jnp.where(hi < 0, hi ^ FLIP, hi), f32)
        idx = (S - 1) - (kk[0, 0] & (S - 1))
        return jnp.clip(idx, 0, S - 1), jax.nn.sigmoid(val)[0:1, 0:1]

    i1, gate1 = decode(k1)
    i2, gate2 = decode(k2)
    c1 = (i1 % RC) // OR
    c2 = (i2 % RC) // OR

    def out_copy(c):
        return pltpu.make_async_copy(ob.at[:, c], o_hbm.at[:, c], sem.at[SEM_OUT + c])

    cp_wd1.wait()
    for c in range(NOC):
        @pl.when(jnp.logical_and(c1 != c, c2 != c))
        def _():
            out_copy(c).start()

    g1 = pl.multiple_of((i1 // 16) * 16, 16)
    g2 = pl.multiple_of((i2 // 16) * 16, 16)
    xsel = jnp.concatenate(
        [jnp.concatenate([h2b[g, pl.ds(r0, 16), :] for g in range(NG)], axis=1)
         for r0 in (g1, g2)], axis=0)
    cp_wg.wait()
    gg = _dot_nt(xsel, wgb[...])
    gg = gg * jax.nn.sigmoid(gg)
    cp_wu.wait()
    act = (gg * _dot_nt(xsel, wub[...])).astype(bf16)

    cp_wd2.wait()
    yy = _dot(act, wdb[...])
    rid = jax.lax.broadcasted_iota(i32, (16, D), 0)
    gbv = modb[4][0:1, :]
    for idx, cc, gate, part in ((i1, c1, gate1, yy[0:16]), (i2, c2, gate2, yy[16:32])):
        upd = jnp.where(rid == idx % 16, part * gate * gbv, 0.0)
        sub = pl.ds(pl.multiple_of(((idx % OR) // 16) * 16, 16), 16)
        ob[idx // RC, cc, sub, :] = (ob[idx // RC, cc, sub, :].astype(f32) + upd).astype(bf16)

    for c in range(NOC):
        @pl.when(jnp.logical_or(c1 == c, c2 == c))
        def _():
            out_copy(c).start()

    for c in range(NOC):
        out_copy(c).wait()


@jax.jit
def pallas_adaLN_cond__ssm_conv_h3__moe_arch_mod__prompt_kernel(
    A_q: jax.Array,
    A_k: jax.Array,
    A_v: jax.Array,
    A_shift_k: jax.Array,
    A_ssm_k: jax.Array,
    A_ssm_D: jax.Array,
    B_x: jax.Array,
    B_w_r: jax.Array,
    B_w_gate: jax.Array,
    B_w_up: jax.Array,
    B_w_down: jax.Array,
    c: jax.Array,
    w_mod: jax.Array,
):
    del B_x
    hbm = pl.BlockSpec(memory_space=pltpu.HBM)
    scratch = [
        pltpu.VMEM((S, D), bf16),
        pltpu.VMEM((S, D), bf16),
        pltpu.VMEM((NG, 128, S), bf16),
        pltpu.VMEM((S, D), bf16),
        pltpu.VMEM((D, 6 * D), bf16),
        pltpu.VMEM((FF, D), bf16),
        pltpu.VMEM((FF, D), bf16),
        pltpu.VMEM((FF, D), bf16),
        pltpu.VMEM((4, D), bf16),
        pltpu.VMEM((NG, 128), bf16),
        pltpu.VMEM((NG, 128), bf16),
        pltpu.VMEM((1, D), bf16),
        pltpu.VMEM((2, BLK + 16, 128), f32),
        pltpu.VMEM((2, BLK, 128), f32),
        pltpu.VMEM((2, S, 128), f32),
        pltpu.VMEM((NG, 2 * NB * R, MT, 8, 128), f32),
        pltpu.VMEM((NG, 2 * NB * R, MT, 8, 128), f32),
        pltpu.VMEM((2, NB * R, 2 * M, 128), bf16),
        pltpu.VMEM((NG, S, 128), f32),
        pltpu.VMEM((NG, S, 128), bf16),
        pltpu.VMEM((S // RC, NOC, OR, D), bf16),
        pltpu.VMEM((R, 2 * M, M), bf16),
        pltpu.VMEM((R, M, 2 * M), bf16),
        pltpu.VMEM((5, 8, D), f32),
        pltpu.VMEM((4, S, 128), f32),
        pltpu.VMEM((S // RC, RC), f32),
        pltpu.SemaphoreType.DMA((NSEM,)),
    ]
    out = pl.pallas_call(
        _kernel,
        out_shape=jax.ShapeDtypeStruct((S // RC, NOC, OR, D), bf16),
        in_specs=[hbm] * 12,
        out_specs=hbm,
        scratch_shapes=scratch,
        compiler_params=pltpu.CompilerParams(
            vmem_limit_bytes=100 * 1024 * 1024, disable_semaphore_checks=True),
    )(
        A_q.reshape(S, D), A_k.reshape(S, D), A_v.reshape(S, D),
        A_shift_k.T, A_ssm_k, A_ssm_D.reshape(NG, 128), B_w_r.reshape(NG, 128),
        B_w_gate.T, B_w_up.T, B_w_down, c, w_mod,
    )
    return out.reshape(1, S, D)
```
